```python
import os as _os
_os.environ.setdefault("JAX_PLATFORMS", "cpu")
import jax
import jax.numpy as jnp

def _softmax(x, axis=-1):
    return jax.nn.softmax(x, axis=axis)
def _gelu(x):
    return jax.nn.gelu(x, approximate=True)
def _silu(x):
    return jax.nn.silu(x)
def _sigmoid(x):
    return jax.nn.sigmoid(x)
def _layernorm(x, axis=-1, eps=1e-5):
    m = jnp.mean(x, axis=axis, keepdims=True)
    v = jnp.var(x, axis=axis, keepdims=True)
    return (x - m) / jnp.sqrt(v + eps)
def _scatter_add(tgt, idx, src, axis=0):
    return tgt.at[idx].add(src)
def _segment_sum(src, seg, n):
    return jax.ops.segment_sum(src, seg, n)
class _Rng:
    def __init__(self, key):
        self._k = key
    def _next(self):
        self._k, sub = jax.random.split(self._k)
        return sub
    def normal(self, shape):
        return jax.random.normal(self._next(), shape, dtype=jnp.bfloat16)
    def randint(self, lo, hi, shape):
        return jax.random.randint(self._next(), shape, lo, hi, dtype=jnp.int32)
    def uniform(self, shape, lo=0.0, hi=1.0):
        return jax.random.uniform(self._next(), shape, jnp.bfloat16, lo, hi)
    def permutation(self, n):
        return jax.random.permutation(self._next(), n)


kernel_name = 'sequential_preLN__sliding_block__glu_gated_swiglu__prompt'

def setup_inputs():
    _rng = _Rng(jax.random.key(int.from_bytes(__import__("os").urandom(4), "little")))
    _w = (lambda a: (lambda t: t.astype(jnp.bfloat16) if jnp.issubdtype(t.dtype, jnp.floating) else t)(jnp.asarray(a)))
    def _A_setup():
        B, S, D = 1, 2048, 640
        return {
            "x": _w((lambda *s: _rng.normal(s) * 0.05)(B, S, D)),
            "wqkv": _w((lambda *s: _rng.normal(s) * 0.05)(D, 3 * D)),
            "wo": _w((lambda *s: _rng.normal(s) * 0.05)(D, D)),
        }
    _A_in = _A_setup()

    def _B_setup():
        B, S, D, F = 1, 2048, 640, 1728
        return {
            "x": _w((lambda *s: _rng.normal(s) * 0.05)(B, S, D)),
            "w1": _w((lambda *s: _rng.normal(s) * 0.1)(D, F) * (2.0 / D) ** 0.5),
            "w3": _w((lambda *s: _rng.normal(s) * 0.1)(D, F) * (2.0 / D) ** 0.5),
            "w2": _w((lambda *s: _rng.normal(s) * 0.1)(F, D) * (2.0 / F) ** 0.5),
        }
    _B_in = _B_setup()

    return {
        "A_x": _A_in["x"],
        "A_wqkv": _A_in["wqkv"],
        "A_wo": _A_in["wo"],
        "B_x": _B_in["x"],
        "B_w1": _B_in["w1"],
        "B_w3": _B_in["w3"],
        "B_w2": _B_in["w2"],
    }

def reference(A_x, A_wqkv, A_wo, B_x, B_w1, B_w3, B_w2):
    def _A_ref(x, wqkv, wo):
        B, S, D = x.shape
        H = 32; Dh = D // H; W = 256
        qkv = (lambda x, *d: x.transpose(*d))((x @ wqkv).reshape(B, S, 3, H, Dh), 2, 0, 3, 1, 4)
        q, k, v = qkv[0], qkv[1], qkv[2]
        scores = jnp.einsum("bhqd,bhkd->bhqk", q, k) * (Dh ** -0.5)
        idx = jnp.arange(S)
        mask = (idx[:, None] - idx[None, :] >= 0) & (idx[:, None] - idx[None, :] < W)
        scores = jnp.where(mask[None, None], scores, -1e9)
        p = _softmax(scores, axis=-1)
        o = jnp.einsum("bhqk,bhkd->bhqd", p, v)
        return (lambda x, *d: x.transpose(*d))(o, 0, 2, 1, 3).reshape(B, S, D) @ wo

    def _B_ref(x, w1, w3, w2):
        gate = jnp.einsum("bsd,df->bsf", x, w1)
        up = jnp.einsum("bsd,df->bsf", x, w3)
        h = _silu(gate) * up
        out = jnp.einsum("bsf,fd->bsd", h, w2)
        return out

    x = A_x
    h = x + _A_ref(_layernorm(x, axis=-1), A_wqkv, A_wo)
    h2 = h + _B_ref(_layernorm(h, axis=-1), B_w1, B_w3, B_w2)
    return h2
```

```python
import functools, math
import jax
import jax.numpy as jnp
from jax import lax
import jax.experimental.pallas as pl
import jax.experimental.pallas.tpu as pltpu

S, D, H, DH, W, F = 2048, 640, 32, 20, 256, 1728
NG = 8
GD = 80
TB = 256
NEG = -1e30
NT = (((1,), (1,)), ((), ()))
f32 = jnp.float32
bf16 = jnp.bfloat16
u32 = jnp.uint32
FM = 1664
QSCALE = DH ** -0.5 * math.log2(math.e)


def _ln(x):
    m = jnp.mean(x, axis=-1, keepdims=True)
    xc = x - m
    v = jnp.mean(xc * xc, axis=-1, keepdims=True)
    return xc * lax.rsqrt(v + 1e-5)


def _group_tile(t, g):
    lo = GD * g
    j0, j1 = lo // 128, (lo + GD - 1) // 128
    a = t[:, 128 * j0:128 * (j0 + 1)]
    if j0 == j1:
        return a
    b = t[:, 128 * j1:128 * (j1 + 1)]
    lane = lax.broadcasted_iota(jnp.int32, a.shape, 1)
    return jnp.where(lane >= lo % 128, a, b)


def _silu_mul(g, u):
    return g * u / (1.0 + jnp.exp(-g))


def kernel(x_ref, xnext_ref, wqkv_hbm, wo_hbm, w1t_hbm, w3t_hbm, w2_hbm, o_ref,
           wqkv_v, wo_v, w1t_v, w3t_v, w2_v, wvt_scr, xn_scr, k_scr, vt_scr, q_scr, p_scr, sems,
           *, cfg):
    i = pl.program_id(0)
    FH = cfg.get("FH", 896)

    def cp(src, dst, s):
        return pltpu.make_async_copy(src, dst, sems.at[s])
    cp_k = cp(wqkv_hbm.at[:, D:2 * D], wqkv_v.at[:, D:2 * D], 0)
    cp_q = cp(wqkv_hbm.at[:, 0:D], wqkv_v.at[:, 0:D], 1)
    cp_v = cp(wqkv_hbm.at[:, 2 * D:3 * D], wqkv_v.at[:, 2 * D:3 * D], 2)
    cp_o = cp(wo_hbm, wo_v, 3)
    cp_1a = cp(w1t_hbm.at[0:FH], w1t_v.at[0:FH], 4)
    cp_3a = cp(w3t_hbm.at[0:FH], w3t_v.at[0:FH], 5)
    cp_1b = cp(w1t_hbm.at[FH:F], w1t_v.at[FH:F], 6)
    cp_3b = cp(w3t_hbm.at[FH:F], w3t_v.at[FH:F], 7)
    cp_2 = cp(w2_hbm, w2_v, 8)

    lane32 = lax.broadcasted_iota(jnp.int32, (32, 128), 1)
    row32 = lax.broadcasted_iota(jnp.int32, (32, 128), 0)
    first_valid = row32 > (lane32 % 32)
    lane16 = lax.broadcasted_iota(jnp.int32, (16, 128), 1)
    bit0_16 = (lane16 // 32) % 2 == 1
    bit1_16 = lane16 >= 64
    sub8 = lax.broadcasted_iota(jnp.int32, (8, 128), 0)
    zero16 = jnp.zeros((16, 128), u32)

    k_u = k_scr.bitcast(u32)
    q_u = q_scr.bitcast(u32)
    p_u = p_scr.bitcast(u32)
    vt_u = vt_scr.bitcast(u32)

    def body(first):
        if first:
            for c_ in (cp_k, cp_q, cp_v, cp_o, cp_1a, cp_3a, cp_1b, cp_3b, cp_2):
                c_.start()
            xn = _ln(x_ref[...].astype(f32)).astype(bf16)
            base = 0
            tbase = 0
            cp_k.wait()
        else:
            xn = xn_scr[...]
            base = pl.multiple_of(i * TB, TB)
            tbase = i * 2
        k = jnp.dot(xn, wqkv_v[:, D:2 * D], preferred_element_type=f32)
        for g in range(NG):
            k_scr[g, pl.ds(base, TB), :] = _group_tile(k, g).astype(bf16)
        if first:
            cp_q.wait()
        q = jnp.dot(xn, wqkv_v[:, 0:D], preferred_element_type=f32) * QSCALE
        for g in range(NG):
            q_scr[g] = _group_tile(q, g).astype(bf16)
        if first:
            cp_v.wait()
            wvt_scr[...] = wqkv_v[:, 2 * D:3 * D].astype(f32).T.astype(bf16)
        vt = lax.dot_general(wvt_scr[...], xn, NT, preferred_element_type=f32)
        ones = jnp.ones((8, TB), f32)
        pieces = []
        for h in range(H):
            st = (DH * h) // 8 * 8
            pieces += [vt[st:st + 24], ones]
        vtp = jnp.concatenate(pieces, axis=0).astype(bf16)
        for a in range(2):
            vt_scr[tbase + a] = vtp[:, 128 * a:128 * (a + 1)]

        def qk_softmax(a, g, slot):
            rel16 = (lane16 + (128 - (GD * g) % 128)) % 128
            for c in range(4):
                q0 = 128 * a + 32 * c
                qu = q_u[g, q0 // 2:q0 // 2 + 16, :]
                wb = []
                for b in range(4):
                    h = b ^ c
                    keep = (rel16 >= DH * h) & (rel16 < DH * (h + 1))
                    wb.append(jnp.where(keep, qu, zero16))
                wq = pltpu.bitcast(jnp.concatenate(wb, axis=0), bf16)
                if first:
                    kc = pltpu.bitcast(k_u[g, 0:q0 // 2 + 16, :], bf16)
                    st = lax.dot_general(kc, wq, NT, preferred_element_type=f32)
                    comb = jnp.where(first_valid, NEG, st[q0:q0 + 32])
                    m = jnp.max(comb, axis=0, keepdims=True)
                    if q0 > 0:
                        m = jnp.maximum(m, jnp.max(st[0:q0], axis=0, keepdims=True))
                        p_scr[slot, c, 0:q0, :] = jnp.exp2(st[0:q0] - m).astype(bf16)
                    p_scr[slot, c, q0:q0 + 32, :] = jnp.exp2(comb - m).astype(bf16)
                else:
                    r0 = pl.multiple_of(i * (TB // 2) + (q0 - W) // 2, 16)
                    kc = pltpu.bitcast(k_u[g, pl.ds(r0, 144), :], bf16)
                    st = lax.dot_general(kc, wq, NT, preferred_element_type=f32)
                    comb = jnp.where(first_valid, st[0:32], st[256:288])
                    bdy = st[32:256]
                    m = jnp.maximum(jnp.max(comb, axis=0, keepdims=True), jnp.max(bdy, axis=0, keepdims=True))
                    pc = jnp.exp2(comb - m)
                    p_scr[slot, c, 0:32, :] = jnp.where(first_valid, pc, 0.0).astype(bf16)
                    p_scr[slot, c, 32:256, :] = jnp.exp2(bdy - m).astype(bf16)
                    p_scr[slot, c, 256:288, :] = jnp.where(first_valid, 0.0, pc).astype(bf16)

        def sel(mask, t, f):
            if t is None and f is None:
                return None
            return jnp.where(mask, zero16 if t is None else t, zero16 if f is None else f)

        def pv(a, g, slot):
            if first:
                nblk = 4 * (a + 1)
                blk = lambda c, j: (p_u[slot, c, 16 * j:16 * j + 16, :]
                                    if j <= 4 * a + c else None)
                tiles = list(range(a + 1))
            else:
                nblk = 12
                blk = lambda c, j: (p_u[slot, c, 16 * (j - c):16 * (j - c) + 16, :]
                                    if c <= j <= c + 8 else None)
                tiles = [tbase + a - 2 + t for t in range(3)]
            outs = [[], [], [], []]
            for j in range(nblk):
                pts = [blk(c, j) for c in range(4)]
                y = [sel(bit0_16, pts[c ^ 1], pts[c]) for c in range(4)]
                for h in range(4):
                    z = sel(bit1_16, y[h ^ 2], y[h])
                    outs[h].append(zero16 if z is None else z)
            on = []
            for h in range(4):
                hh = 4 * g + h
                pth = pltpu.bitcast(jnp.concatenate(outs[h], axis=0), bf16)
                vth = pltpu.bitcast(jnp.concatenate([vt_u[t, 16 * hh:16 * hh + 16, :] for t in tiles], axis=1), bf16)
                ot = jnp.dot(vth, pth, preferred_element_type=f32)
                r = 1.0 / ot[24:32]
                on.append([ot[0:8] * r, ot[8:16] * r, ot[16:24] * r])
            return [on[0][0], on[0][1], jnp.where(sub8 < 4, on[0][2], on[1][0]), on[1][1], on[1][2],
                    on[2][0], on[2][1], jnp.where(sub8 < 4, on[2][2], on[3][0]), on[3][1], on[3][2]]

        def wo_ln2(a, m_all):
            mt = jnp.concatenate(m_all, axis=0).T
            col = lax.broadcasted_iota(jnp.int32, (32, D), 1)
            hb0 = (col // DH) % 2 == 1
            hb1 = (col // (2 * DH)) % 2 == 1
            rb = [mt[32 * b:32 * (b + 1)] for b in range(4)]
            y = [jnp.where(hb0, rb[c ^ 1], rb[c]) for c in range(4)]
            z = [jnp.where(hb1, y[c ^ 2], y[c]) for c in range(4)]
            o = jnp.concatenate(z, axis=0).astype(bf16)
            h1 = x_ref[128 * a:128 * (a + 1), :].astype(f32) + jnp.dot(o, wo_v[...], preferred_element_type=f32)
            return h1, _ln(h1).astype(bf16)

        def gu(hn, lo, hi):
            gate = lax.dot_general(hn, w1t_v[lo:hi, :], NT, preferred_element_type=f32)
            up = lax.dot_general(hn, w3t_v[lo:hi, :], NT, preferred_element_type=f32)
            return _silu_mul(gate, up).astype(bf16)

        def gu_tail(hn):
            wt = jnp.concatenate([w1t_v[FM:F, :], w3t_v[FM:F, :]], axis=0)
            t = lax.dot_general(hn, wt, NT, preferred_element_type=f32)
            return _silu_mul(t, pltpu.roll(t, 64, 1))[:, 0:64].astype(bf16)

        units = [(a, g) for a in range(2) for g in range(NG)]
        NS = cfg.get("NS", 2)
        LAG = cfg.get("LAG", 1)
        WO0 = cfg.get("WO0", 10)
        m_all = [[], []]
        h1 = [None, None]
        hn = [None, None]
        hid0 = []
        CH = cfg.get("CH", 256)
        chunks = [(lo, min(lo + CH, FM)) for lo in range(0, FM, CH)]
        for n in range(16 + LAG):
            if n < 16:
                qk_softmax(*units[n], n % NS)
            elif n == 16 + LAG - 1:
                if first:
                    cp_1a.wait()
                    cp_3a.wait()
                hid0.append(gu(hn[0], *chunks[0]))
            if n >= LAG:
                a, g = units[n - LAG]
                m_all[a] += pv(a, g, (n - LAG) % NS)
                if n - LAG == WO0:
                    if first:
                        cp_o.wait()
                    h1[0], hn[0] = wo_ln2(0, m_all[0])
        hid0.append(gu(hn[0], *chunks[1]))
        h1[1], hn[1] = wo_ln2(1, m_all[1])
        waited = False
        for lo, hi in chunks[2:]:
            if first and hi > FH and not waited:
                cp_1b.wait()
                cp_3b.wait()
                waited = True
            hid0.append(gu(hn[0], lo, hi))
        hid0.append(gu_tail(hn[0]))
        hid1 = [gu(hn[1], lo, hi) for lo, hi in chunks] + [gu_tail(hn[1])]
        xn_scr[...] = _ln(xnext_ref[...].astype(f32)).astype(bf16)
        if first:
            cp_2.wait()
        for a, hid in ((0, hid0), (1, hid1)):
            out = h1[a] + jnp.dot(jnp.concatenate(hid, axis=1), w2_v[...], preferred_element_type=f32)
            o_ref[128 * a:128 * (a + 1), :] = out.astype(o_ref.dtype)

    pl.when(i == 0)(lambda: body(True))
    pl.when(i > 0)(lambda: body(False))


@jax.jit
def pallas_sequential_preLN__sliding_block__glu_gated_swiglu__prompt_kernel(A_x, A_wqkv, A_wo, B_x, B_w1, B_w3, B_w2):
    cfg = dict(WO0=12)
    x = A_x.reshape(S, D)
    nb = S // TB
    hbm = pl.BlockSpec(memory_space=pl.ANY)
    out = pl.pallas_call(
        functools.partial(kernel, cfg=cfg),
        grid=(nb,),
        in_specs=[
            pl.BlockSpec((TB, D), lambda i: (i, 0)),
            pl.BlockSpec((TB, D), lambda i: (jnp.minimum(i + 1, nb - 1), 0)),
            hbm, hbm, hbm, hbm, hbm,
        ],
        out_specs=pl.BlockSpec((TB, D), lambda i: (i, 0)),
        out_shape=jax.ShapeDtypeStruct((S, D), bf16),
        scratch_shapes=[
            pltpu.VMEM((D, 3 * D), bf16),
            pltpu.VMEM((D, D), bf16),
            pltpu.VMEM((F, D), bf16),
            pltpu.VMEM((F, D), bf16),
            pltpu.VMEM((F, D), bf16),
            pltpu.VMEM((D, D), bf16),
            pltpu.VMEM((TB, D), bf16),
            pltpu.VMEM((NG, S, 128), bf16),
            pltpu.VMEM((S // 128, H * 32, 128), bf16),
            pltpu.VMEM((NG, TB, 128), bf16),
            pltpu.VMEM((cfg.get("NS", 2), 4, 288, 128), bf16),
            pltpu.SemaphoreType.DMA((9,)),
        ],
        compiler_params=pltpu.CompilerParams(
            dimension_semantics=("arbitrary",),
            vmem_limit_bytes=100 * 1024 * 1024),
    )(x, x, A_wqkv, A_wo, B_w1.T, B_w3.T, B_w2)
    return out.reshape(1, S, D)
```

```python
import functools, math
import jax
import jax.numpy as jnp
from jax import lax
import jax.experimental.pallas as pl
import jax.experimental.pallas.tpu as pltpu

S, D, H, DH, W, F = 2048, 640, 32, 20, 256, 1728
NG = 8
GD = 80
TB = 256
NA = TB // 128
NB = S // TB
NEG = -1e30
SAFE = 60.0
NT = (((1,), (1,)), ((), ()))
f32 = jnp.float32
bf16 = jnp.bfloat16
u32 = jnp.uint32
FM = 1664
QSCALE = DH ** -0.5 * math.log2(math.e)


def _ln(x):
    m = jnp.mean(x, axis=-1, keepdims=True)
    xc = x - m
    v = jnp.mean(xc * xc, axis=-1, keepdims=True)
    return xc * lax.rsqrt(v + 1e-5)


def _group_tile(t, g):
    lo = GD * g
    j0, j1 = lo // 128, (lo + GD - 1) // 128
    a = t[:, 128 * j0:128 * (j0 + 1)]
    if j0 == j1:
        return a
    b = t[:, 128 * j1:128 * (j1 + 1)]
    lane = lax.broadcasted_iota(jnp.int32, a.shape, 1)
    return jnp.where(lane >= lo % 128, a, b)


def kernel(x_hbm, wqkv_hbm, wo_hbm, w1t_hbm, w3t_hbm, w2_hbm, o_hbm,
           x_v, o_v, wqkv_v, wo_v, w1t_v, w3t_v, w2_v, wvt_scr, xn_scr, k_scr, vt_scr, q_scr, p_scr,
           m_scr, sems, osem, *, cfg):
    FH = cfg.get("FH", 768)

    def silu_mul(g, u):
        if cfg.get("TANH", 0):
            return (g * u) * (0.5 * jnp.tanh(0.5 * g) + 0.5)
        return g * u / (1.0 + jnp.exp(-g))

    def cp(src, dst, s):
        return pltpu.make_async_copy(src, dst, sems.at[s])
    cp_x0 = cp(x_hbm.at[0:TB], x_v.at[0:TB], 0)
    cp_k = cp(wqkv_hbm.at[:, D:2 * D], wqkv_v.at[:, D:2 * D], 1)
    cp_q = cp(wqkv_hbm.at[:, 0:D], wqkv_v.at[:, 0:D], 2)
    cp_v = cp(wqkv_hbm.at[:, 2 * D:3 * D], wqkv_v.at[:, 2 * D:3 * D], 3)
    cp_o = cp(wo_hbm, wo_v, 4)
    cp_1 = cp(w1t_hbm.at[0:FH], w1t_v.at[0:FH], 4)
    cp_3 = cp(w3t_hbm.at[0:FH], w3t_v.at[0:FH], 4)
    cp_1b = cp(w1t_hbm.at[FH:F], w1t_v.at[FH:F], 5)
    cp_3b = cp(w3t_hbm.at[FH:F], w3t_v.at[FH:F], 5)
    cp_xn = cp(x_hbm.at[TB:2 * TB], x_v.at[TB:2 * TB], 6)
    cp_2 = cp(w2_hbm, w2_v, 6)
    cp_xr = cp(x_hbm.at[2 * TB:S], x_v.at[2 * TB:S], 7)

    allc = [cp_x0, cp_k, cp_q, cp_v, cp_o, cp_1, cp_3, cp_1b, cp_3b, cp_xn, cp_2, cp_xr]
    if cfg.get("KFIRST"):
        allc[0], allc[1] = allc[1], allc[0]
    early_starts, late_starts = allc[:cfg.get("N0", 12)], allc[cfg.get("N0", 12):]

    def out_cp(row0, a):
        r = row0 + 128 * a
        return pltpu.make_async_copy(o_v.at[pl.ds(r, 128)], o_hbm.at[pl.ds(r, 128)], osem)

    lane32 = lax.broadcasted_iota(jnp.int32, (32, 128), 1)
    row32 = lax.broadcasted_iota(jnp.int32, (32, 128), 0)
    first_valid = row32 > (lane32 % 32)
    lane16 = lax.broadcasted_iota(jnp.int32, (16, 128), 1)
    bit0_16 = (lane16 // 32) % 2 == 1
    bit1_16 = lane16 >= 64
    sub8 = lax.broadcasted_iota(jnp.int32, (8, 128), 0)
    zero16 = jnp.zeros((16, 128), u32)
    k_u = k_scr.bitcast(u32)
    q_u = q_scr.bitcast(u32)
    p_u = p_scr.bitcast(u32)
    vt_u = vt_scr.bitcast(u32)
    NS = cfg.get('NS', 4)
    nw = []

    def body(first, i, redo):
        if first:
            base, hbase, tbase = 0, 0, 0
        else:
            base = pl.multiple_of(i * TB, TB)
            hbase = i * (TB // 2)
            tbase = i * NA

        def waits(cps, start=()):
            if first:
                def w():
                    for c_ in cps:
                        c_.wait()
                    for c_ in start:
                        c_.start()
                if cfg.get("PROF"):
                    with jax.named_scope("wait%d" % len(nw)):
                        pl.when(jnp.logical_not(redo))(w)
                    nw.append(0)
                else:
                    pl.when(jnp.logical_not(redo))(w)

        def proj_k(xn):
            k = jnp.dot(xn, wqkv_v[:, D:2 * D], preferred_element_type=f32)
            for g in range(NG):
                k_scr[g, pl.ds(base, TB), :] = _group_tile(k, g).astype(bf16)

        def proj_q(xn):
            q = jnp.dot(xn, wqkv_v[:, 0:D], preferred_element_type=f32) * QSCALE
            for g in range(NG):
                q_scr[g] = _group_tile(q, g).astype(bf16)

        def proj_v(xn):
            vt = lax.dot_general(wvt_scr[...], xn, NT, preferred_element_type=f32)
            ones = jnp.ones((8, TB), f32)
            pieces = []
            for h in range(H):
                st = (DH * h) // 8 * 8
                pieces += [vt[st:st + 24], ones]
            vtp = jnp.concatenate(pieces, axis=0).astype(bf16)
            for a in range(NA):
                vt_scr[tbase + a] = vtp[:, 128 * a:128 * (a + 1)]

        def qk(a, g, slot, mabs):
            rel16 = (lane16 + (128 - (GD * g) % 128)) % 128
            for c in range(4):
                q0 = 128 * a + 32 * c
                un = (a * NG + g) * 4 + c
                qu = q_u[g, q0 // 2:q0 // 2 + 16, :]
                wb = []
                for b in range(4):
                    h = b ^ c
                    keep = (rel16 >= DH * h) & (rel16 < DH * (h + 1))
                    wb.append(jnp.where(keep, qu, zero16))
                wq = pltpu.bitcast(jnp.concatenate(wb, axis=0), bf16)
                mref = jnp.where(redo, m_scr[un], 0.0)
                if first:
                    kc = pltpu.bitcast(k_u[g, 0:q0 // 2 + 16, :], bf16)
                    st = lax.dot_general(kc, wq, NT, preferred_element_type=f32)
                    comb = jnp.where(first_valid, NEG, st[q0:q0 + 32])
                    sc = comb if q0 == 0 else jnp.concatenate([st[0:q0], comb], axis=0)
                    p_scr[slot, c, 0:q0 + 32, :] = jnp.exp2(sc - mref).astype(bf16)
                else:
                    r0 = pl.multiple_of(hbase + (q0 - W) // 2, 16)
                    kc = pltpu.bitcast(k_u[g, pl.ds(r0, 144), :], bf16)
                    st = lax.dot_general(kc, wq, NT, preferred_element_type=f32)
                    comb = jnp.where(first_valid, st[0:32], st[256:288])
                    sc = jnp.concatenate([st[32:256], comb], axis=0)
                    pc = jnp.exp2(comb - mref)
                    p_scr[slot, c, 0:32, :] = jnp.where(first_valid, pc, 0.0).astype(bf16)
                    p_scr[slot, c, 32:256, :] = jnp.exp2(st[32:256] - mref).astype(bf16)
                    p_scr[slot, c, 256:288, :] = jnp.where(first_valid, 0.0, pc).astype(bf16)
                m = jnp.max(sc, axis=0, keepdims=True)
                m_scr[un] = m
                am = jnp.abs(m)
                mabs = am if mabs is None else jnp.maximum(mabs, am)
            return mabs

        def sel(mask, t, f):
            if t is None and f is None:
                return None
            return jnp.where(mask, zero16 if t is None else t, zero16 if f is None else f)

        def pv(a, g, slot):
            if first:
                nblk = 4 * (a + 1)
                blk = lambda c, j: (p_u[slot, c, 16 * j:16 * j + 16, :] if j <= 4 * a + c else None)
                tiles = list(range(a + 1))
            else:
                nblk = 12
                blk = lambda c, j: (p_u[slot, c, 16 * (j - c):16 * (j - c) + 16, :] if c <= j <= c + 8 else None)
                tiles = [tbase + a - 2 + t for t in range(3)]
            outs = [[], [], [], []]
            for j in range(nblk):
                pts = [blk(c, j) for c in range(4)]
                y = [sel(bit0_16, pts[c ^ 1], pts[c]) for c in range(4)]
                for h in range(4):
                    z = sel(bit1_16, y[h ^ 2], y[h])
                    outs[h].append(zero16 if z is None else z)
            ots = [None] * 4
            for ti, t in enumerate(tiles):
                for h in range(4):
                    hh = 4 * g + h
                    pth = pltpu.bitcast(jnp.concatenate(outs[h][4 * ti:4 * ti + 4], axis=0), bf16)
                    vth = pltpu.bitcast(vt_u[t, 16 * hh:16 * hh + 16, :], bf16)
                    d = jnp.dot(vth, pth, preferred_element_type=f32)
                    ots[h] = d if ots[h] is None else ots[h] + d
            on = []
            for h in range(4):
                ot = ots[h]
                r = 1.0 / ot[24:32]
                on.append([ot[0:8] * r, ot[8:16] * r, ot[16:24] * r])
            return [on[0][0], on[0][1], jnp.where(sub8 < 4, on[0][2], on[1][0]), on[1][1], on[1][2],
                    on[2][0], on[2][1], jnp.where(sub8 < 4, on[2][2], on[3][0]), on[3][1], on[3][2]]

        def wo_ln2(a, m_all):
            mt = jnp.concatenate(m_all, axis=0).T
            col = lax.broadcasted_iota(jnp.int32, (32, D), 1)
            hb0 = (col // DH) % 2 == 1
            hb1 = (col // (2 * DH)) % 2 == 1
            rb = [mt[32 * b:32 * (b + 1)] for b in range(4)]
            y = [jnp.where(hb0, rb[c ^ 1], rb[c]) for c in range(4)]
            z = [jnp.where(hb1, y[c ^ 2], y[c]) for c in range(4)]
            o = jnp.concatenate(z, axis=0).astype(bf16)
            h1 = (x_v[pl.ds(base + 128 * a, 128), :].astype(f32)
                  + jnp.dot(o, wo_v[...], preferred_element_type=f32))
            return h1, _ln(h1).astype(bf16)

        def gu(hn, lo, hi, tie=None):
            if lo == FM:
                wt = jnp.concatenate([w1t_v[FM:F, :], w3t_v[FM:F, :]], axis=0)
                t = lax.dot_general(hn, wt, NT, preferred_element_type=f32)
                return silu_mul(t, pltpu.roll(t, 64, 1))[:, 0:64].astype(bf16)
            gate = lax.dot_general(hn, w1t_v[lo:hi, :], NT, preferred_element_type=f32)
            up = lax.dot_general(hn, w3t_v[lo:hi, :], NT, preferred_element_type=f32)
            r = silu_mul(gate, up)
            if tie is not None:
                r = jnp.where(i > NB, tie, r)
            return r.astype(bf16)

        CH = cfg.get("CH", 128)
        chunks = [(lo, min(lo + CH, FM)) for lo in range(0, FM, CH)] + [(FM, F)]
        nch = len(chunks)
        NU = NA * NG
        WOD = cfg.get("WOD", 4)
        G0 = cfg.get("G0", 1)
        G1 = cfg.get("G1", 2)
        if first:
            waits([cp_x0], late_starts)
            xn = _ln(x_v[0:TB, :].astype(f32)).astype(bf16)
            waits([cp_k])
            proj_k(xn)
            LAG = cfg.get("LAGF", 1)
            WOD = cfg.get("WODF", 4)
            if cfg.get("QV", 0):
                waits([cp_q])
                proj_q(xn)
                waits([cp_v])
                wvt_scr[...] = wqkv_v[:, 2 * D:3 * D].astype(f32).T.astype(bf16)
                pre = [("pj_v",)]
            else:
                waits([cp_q, cp_v])
                wvt_scr[...] = wqkv_v[:, 2 * D:3 * D].astype(f32).T.astype(bf16)
                proj_q(xn)
                proj_v(xn)
                pre = []
        else:
            xn = xn_scr[i % 2]
            proj_k(xn)
            proj_q(xn)
            proj_v(xn)
            LAG = 1
            pre = []

        order = []
        for n in range(NU + LAG):
            if n < NU:
                order.append(("qk", n))
            elif n == NU + LAG - 1:
                order += [("gu", 0, j) for j in range(G0)]
            if n == LAG - 1:
                order += pre
            if n >= LAG:
                order.append(("pv", n - LAG))
                if n - LAG - WOD == NG - 1:
                    order.append(("wo", 0))
        order += [("gu", 0, j) for j in range(G0, G1)]
        order.append(("wo", 1))
        nh = sum(1 for lo, hi in chunks if hi <= FH) if first else nch
        order += [("gu", 0, j) for j in range(G1, nh)] + [("gu", 1, j) for j in range(nh)]
        order += [("gu", 0, j) for j in range(nh, nch)] + [("gu", 1, j) for j in range(nh, nch)]
        order += [("dn", 0), ("ln1",), ("dn", 1)]

        m_all = [[] for _ in range(NA)]
        h1 = [None] * NA
        hn = [None] * NA
        hid = [[] for _ in range(NA)]
        waited = set()
        mabs = None
        xnf = None
        done = None

        def wait_once(name, cps):
            if name not in waited:
                waited.add(name)
                waits(cps)

        for t in order:
            if t[0] == "qk":
                mabs = qk(t[1] // NG, t[1] % NG, t[1] % NS, mabs)
            elif t[0] == "pv":
                m_all[t[1] // NG] += pv(t[1] // NG, t[1] % NG, t[1] % NS)
            elif t[0] == "pj_v":
                proj_v(xn)
            elif t[0] == "wo":
                wait_once("f", [cp_o, cp_1, cp_3])
                h1[t[1]], hn[t[1]] = wo_ln2(t[1], m_all[t[1]])
            elif t[0] == "gu":
                wait_once("f", [cp_1, cp_3])
                if chunks[t[2]][1] > FH:
                    wait_once("fb", [cp_1b, cp_3b])
                tie = None
                TJ = cfg.get("TJ", 3)
                if cfg.get("TIE", 1) and not first and t[1] == 1 and TJ <= t[2] < TJ + 10:
                    if xnf is None:
                        nxt = pl.multiple_of(jnp.minimum(i + 1, NB - 1) * TB, TB)
                        xnf = _ln(x_v[pl.ds(nxt, TB), :].astype(f32))
                        xn_scr[(i + 1) % 2] = xnf.astype(bf16)
                    jj = t[2] - TJ
                    tie = xnf[128 * (jj // 5):128 * (jj // 5 + 1), 128 * (jj % 5):128 * (jj % 5 + 1)]
                hid[t[1]].append(gu(hn[t[1]], *chunks[t[2]], tie=tie))
            elif t[0] == "ln1" and xnf is None:
                nxt = pl.multiple_of(jnp.minimum(i + 1, NB - 1) * TB, TB)
                xn_scr[(i + 1) % 2] = _ln(x_v[pl.ds(nxt, TB), :].astype(f32)).astype(bf16)
            elif t[0] == "dn":
                wait_once("d", [cp_xn, cp_2])
                a = t[1]
                hcat = jnp.concatenate(hid[a], axis=1)
                out = h1[a] + jnp.dot(hcat, w2_v[...], preferred_element_type=f32)
                o_v[pl.ds(base + 128 * a, 128), :] = out.astype(bf16)
                if done is None:
                    ok = jnp.where(mabs <= SAFE, 1.0, 0.0)
                    done = jnp.logical_or(redo, jnp.min(ok) > 0.5)
                pl.when(done)(out_cp(base, a).start)
        waits([cp_xr])
        return done

    for c_ in early_starts:
        c_.start()

    def step(first, carry):
        i, r = carry
        done = body(first, i, r == 1)
        return jnp.where(done, i + 1, i), jnp.where(done, 0, 1)

    with jax.named_scope("first"):
        lax.while_loop(lambda c: c[0] < 1, functools.partial(step, True), (jnp.int32(0), jnp.int32(0)))
    with jax.named_scope("steady"):
        lax.while_loop(lambda c: c[0] < NB, functools.partial(step, False), (jnp.int32(1), jnp.int32(0)))
    pltpu.make_async_copy(o_v, o_hbm, osem).wait()


@jax.jit
def pallas_sequential_preLN__sliding_block__glu_gated_swiglu__prompt_kernel(A_x, A_wqkv, A_wo, B_x, B_w1, B_w3, B_w2):
    cfg = dict(TANH=1,FH=640,LAGF=3,QV=1)
    x = A_x.reshape(S, D)
    hbm = pl.BlockSpec(memory_space=pl.ANY)
    out = pl.pallas_call(
        functools.partial(kernel, cfg=cfg),
        in_specs=[hbm] * 6,
        out_specs=hbm,
        out_shape=jax.ShapeDtypeStruct((S, D), bf16),
        scratch_shapes=[
            pltpu.VMEM((S, D), bf16),
            pltpu.VMEM((S, D), bf16),
            pltpu.VMEM((D, 3 * D), bf16),
            pltpu.VMEM((D, D), bf16),
            pltpu.VMEM((F, D), bf16),
            pltpu.VMEM((F, D), bf16),
            pltpu.VMEM((F, D), bf16),
            pltpu.VMEM((D, D), bf16),
            pltpu.VMEM((2, TB, D), bf16),
            pltpu.VMEM((NG, S, 128), bf16),
            pltpu.VMEM((S // 128, H * 32, 128), bf16),
            pltpu.VMEM((NG, TB, 128), bf16),
            pltpu.VMEM((cfg.get('NS', 4), 4, 288, 128), bf16),
            pltpu.VMEM((NA * NG * 4, 1, 128), f32),
            pltpu.SemaphoreType.DMA((8,)),
            pltpu.SemaphoreType.DMA(()),
        ],
        compiler_params=pltpu.CompilerParams(
            vmem_limit_bytes=100 * 1024 * 1024),
    )(x, A_wqkv, A_wo, B_w1.T, B_w3.T, B_w2)
    return out.reshape(1, S, D)
```

```python
import functools
import math

import jax
import jax.numpy as jnp
from jax import lax
import jax.experimental.pallas as pl
import jax.experimental.pallas.tpu as pltpu

S, D, H, DH, W, F = 2048, 640, 32, 20, 256, 1728
NG = 8
GD = 80
TB = 256
NA = TB // 128
NB = S // TB
NU = NA * NG
NEG = -1e30
SAFE = 40.0
NT = (((1,), (1,)), ((), ()))
f32 = jnp.float32
bf16 = jnp.bfloat16
u32 = jnp.uint32
FM = 1664
FH = 896
CA, CB = 1024, 512
QSCALE = DH ** -0.5 * math.log2(math.e)


def _ln(x):
    m = jnp.mean(x, axis=-1, keepdims=True)
    xc = x - m
    v = jnp.mean(xc * xc, axis=-1, keepdims=True)
    return xc * lax.rsqrt(v + 1e-5)


def _group_tile(t, g):
    lo = GD * g
    j0, j1 = lo // 128, (lo + GD - 1) // 128
    a = t[:, 128 * j0:128 * (j0 + 1)]
    if j0 == j1:
        return a
    b = t[:, 128 * j1:128 * (j1 + 1)]
    lane = lax.broadcasted_iota(jnp.int32, a.shape, 1)
    return jnp.where(lane >= lo % 128, a, b)


def _silu_mul(g, u):
    return (g * u) * (0.5 * jnp.tanh(0.5 * g) + 0.5)


def _dot(a, b):
    return jnp.dot(a, b, preferred_element_type=f32)


def _dot_nt(a, b):
    return lax.dot_general(a, b, NT, preferred_element_type=f32)


def _dot_bal(lhs, w, nsplit):
    n = w.shape[1] - 128
    r = lhs.shape[0] // nsplit
    main = _dot(lhs, w[:, :n])
    last = [_dot(lhs[r * u:r * (u + 1)], w[:, n:]) for u in range(nsplit)]
    return jnp.concatenate([main, jnp.concatenate(last, axis=0)], axis=1)


def _kernel(x_hbm, wqkv_hbm, wo_hbm, w1t_hbm, w3t_hbm, w2_hbm, o_hbm,
            x_v, o_v, wqkv_v, wo_v, w1t_v, w3t_v, w2_v, wvt_scr, xn_scr, k_scr, vt_scr, q_scr, p_scr,
            m_scr, sems, osem):
    def cp(src, dst, s):
        return pltpu.make_async_copy(src, dst, sems.at[s])

    groups = {
        "x0": [cp(x_hbm.at[0:TB], x_v.at[0:TB], 0)],
        "a": [cp(wqkv_hbm.at[:, CA:2 * D], wqkv_v.at[:, CA:2 * D], 1)],
        "b": [cp(wqkv_hbm.at[:, CB:CA], wqkv_v.at[:, CB:CA], 2)],
        "c": [cp(wqkv_hbm.at[:, 0:CB], wqkv_v.at[:, 0:CB], 3)],
        "vo": [cp(wqkv_hbm.at[:, 2 * D:3 * D], wqkv_v.at[:, 2 * D:3 * D], 4), cp(wo_hbm, wo_v, 4)],
        "fa": [cp(w1t_hbm.at[0:FH], w1t_v.at[0:FH], 5), cp(w3t_hbm.at[0:FH], w3t_v.at[0:FH], 5)],
        "fb": [cp(w1t_hbm.at[FH:F], w1t_v.at[FH:F], 6), cp(w3t_hbm.at[FH:F], w3t_v.at[FH:F], 6),
               cp(x_hbm.at[TB:2 * TB], x_v.at[TB:2 * TB], 6)],
        "w2": [cp(w2_hbm, w2_v, 7)],
        "xr": [cp(x_hbm.at[2 * TB:S], x_v.at[2 * TB:S], 8)],
    }

    def out_cp(r, c0, c1):
        return pltpu.make_async_copy(o_v.at[pl.ds(r, 128), c0:c1], o_hbm.at[pl.ds(r, 128), c0:c1], osem)

    lane32 = lax.broadcasted_iota(jnp.int32, (32, 128), 1)
    row32 = lax.broadcasted_iota(jnp.int32, (32, 128), 0)
    old_valid = row32 > (lane32 % 32)
    lane16 = lax.broadcasted_iota(jnp.int32, (16, 128), 1)
    bit0 = (lane16 // 32) % 2 == 1
    bit1 = lane16 >= 64
    sub8 = lax.broadcasted_iota(jnp.int32, (8, 128), 0)
    zero16 = jnp.zeros((16, 128), u32)
    k_u = k_scr.bitcast(u32)
    q_u = q_scr.bitcast(u32)
    p_u = p_scr.bitcast(u32)
    vt_u = vt_scr.bitcast(u32)
    chunks = [(lo, lo + 128) for lo in range(0, FM, 128)] + [(FM, F)]
    nch = len(chunks)

    def body(first, i, redo):
        if first:
            base, hbase, tbase = 0, 0, 0
        else:
            base = pl.multiple_of(i * TB, TB)
            hbase = i * (TB // 2)
            tbase = i * NA

        def put_k(k):
            for g in range(NG):
                k_scr[g, pl.ds(base, TB), :] = _group_tile(k, g).astype(bf16)

        def put_q(q):
            q = q * QSCALE
            for g in range(NG):
                q_scr[g] = _group_tile(q, g).astype(bf16)

        def proj_v(xn):
            vt = _dot_nt(wvt_scr[...], xn)
            ones = jnp.ones((8, TB), f32)
            pieces = []
            for h in range(H):
                st = (DH * h) // 8 * 8
                pieces += [vt[st:st + 24], ones]
            vtp = jnp.concatenate(pieces, axis=0).astype(bf16)
            for a in range(NA):
                vt_scr[tbase + a] = vtp[:, 128 * a:128 * (a + 1)]

        def qk(n, mabs):
            a, g = n // NG, n % NG
            rel = (lane16 + (128 - (GD * g) % 128)) % 128
            for c in range(4):
                q0 = 128 * a + 32 * c
                un = n * 4 + c
                qu = q_u[g, q0 // 2:q0 // 2 + 16, :]
                wb = []
                for b in range(4):
                    h = b ^ c
                    wb.append(jnp.where((rel >= DH * h) & (rel < DH * (h + 1)), qu, zero16))
                wq = pltpu.bitcast(jnp.concatenate(wb, axis=0), bf16)
                mref = jnp.where(redo, m_scr[un], 0.0)
                if first:
                    st = _dot_nt(pltpu.bitcast(k_u[g, 0:q0 // 2 + 16, :], bf16), wq)
                    diag = jnp.where(old_valid, NEG, st[q0:q0 + 32])
                    sc = diag if q0 == 0 else jnp.concatenate([st[0:q0], diag], axis=0)
                    p_scr[n, c, 0:q0 + 32, :] = jnp.exp2(sc - mref).astype(bf16)
                else:
                    r0 = pl.multiple_of(hbase + (q0 - W) // 2, 16)
                    st = _dot_nt(pltpu.bitcast(k_u[g, pl.ds(r0, 144), :], bf16), wq)
                    edge = jnp.where(old_valid, st[0:32], st[256:288])
                    sc = jnp.concatenate([st[32:256], edge], axis=0)
                    pe = jnp.exp2(edge - mref)
                    p_scr[n, c, 0:32, :] = jnp.where(old_valid, pe, 0.0).astype(bf16)
                    p_scr[n, c, 32:256, :] = jnp.exp2(st[32:256] - mref).astype(bf16)
                    p_scr[n, c, 256:288, :] = jnp.where(old_valid, 0.0, pe).astype(bf16)
                m = jnp.max(sc, axis=0, keepdims=True)
                m_scr[un] = m
                am = jnp.abs(m)
                mabs = am if mabs is None else jnp.maximum(mabs, am)
            return mabs

        def sel(mask, t, f):
            if t is None and f is None:
                return None
            return jnp.where(mask, zero16 if t is None else t, zero16 if f is None else f)

        def pv(n):
            a, g = n // NG, n % NG
            if first:
                nblk = 4 * (a + 1)
                blk = lambda c, j: (p_u[n, c, 16 * j:16 * j + 16, :] if j <= 4 * a + c else None)
                tiles = list(range(a + 1))
            else:
                nblk = 12
                blk = lambda c, j: (p_u[n, c, 16 * (j - c):16 * (j - c) + 16, :] if c <= j <= c + 8 else None)
                tiles = [tbase + a - 2 + t for t in range(3)]
            outs = [[], [], [], []]
            for j in range(nblk):
                pts = [blk(c, j) for c in range(4)]
                y = [sel(bit0, pts[c ^ 1], pts[c]) for c in range(4)]
                for h in range(4):
                    z = sel(bit1, y[h ^ 2], y[h])
                    outs[h].append(zero16 if z is None else z)
            ots = [None] * 4
            for ti, t in enumerate(tiles):
                for h in range(4):
                    hh = 4 * g + h
                    pth = pltpu.bitcast(jnp.concatenate(outs[h][4 * ti:4 * ti + 4], axis=0), bf16)
                    d = _dot(pltpu.bitcast(vt_u[t, 16 * hh:16 * hh + 16, :], bf16), pth)
                    ots[h] = d if ots[h] is None else ots[h] + d
            on = []
            for h in range(4):
                r = 1.0 / ots[h][24:32]
                on.append([ots[h][0:8] * r, ots[h][8:16] * r, ots[h][16:24] * r])
            return [on[0][0], on[0][1], jnp.where(sub8 < 4, on[0][2], on[1][0]), on[1][1], on[1][2],
                    on[2][0], on[2][1], jnp.where(sub8 < 4, on[2][2], on[3][0]), on[3][1], on[3][2]]

        def wo(a, ot_rows):
            mt = jnp.concatenate(ot_rows, axis=0).T
            col = lax.broadcasted_iota(jnp.int32, (32, D), 1)
            hb0 = (col // DH) % 2 == 1
            hb1 = (col // (2 * DH)) % 2 == 1
            rb = [mt[32 * b:32 * (b + 1)] for b in range(4)]
            y = [jnp.where(hb0, rb[c ^ 1], rb[c]) for c in range(4)]
            z = [jnp.where(hb1, y[c ^ 2], y[c]) for c in range(4)]
            o = jnp.concatenate(z, axis=0).astype(bf16)
            return x_v[pl.ds(base + 128 * a, 128), :].astype(f32) + _dot(o, wo_v[...])

        def gu_mm(hn, j):
            lo, hi = chunks[j]
            if lo == FM:
                return (_dot_nt(hn, jnp.concatenate([w1t_v[FM:F, :], w3t_v[FM:F, :]], axis=0)),)
            return _dot_nt(hn, w1t_v[lo:hi, :]), _dot_nt(hn, w3t_v[lo:hi, :])

        def act(gu_, tie):
            if len(gu_) == 1:
                t = gu_[0]
                return _silu_mul(t, pltpu.roll(t, 64, 1))[:, 0:64].astype(bf16)
            r = _silu_mul(*gu_)
            if tie is not None:
                r = jnp.where(i > NB, tie, r)
            return r.astype(bf16)

        G = lambda a, js: [("gu", a, j) for j in js]
        if first:
            nh = FH // 128
            order = [("start",), ("wait", "x0"), ("ln0",), ("wait", "a"), ("pa",), ("wait", "b"), ("pb",),
                     ("wait", "c"), ("pc",)]
            order += [("qk", n) for n in list(range(NG, NU - 2)) + list(range(NG))]
            order += [("wait", "vo"), ("wvt",), ("qk", NU - 2), ("qk", NU - 1), ("pjv",)]
            order += [("pv", n) for n in range(NU)]
            order += [("wo", 0), ("ln2", 0), ("wo", 1), ("wait", "fa"), ("ln2", 1)]
            order += G(0, range(nh)) + G(1, range(nh - 1)) + [("gm", 1, nh - 1), ("wait", "fb"), ("ac", 1, nh - 1)]
            order += G(0, [nch - 1]) + G(1, [nch - 1])
            order += G(0, range(nh, nch - 1)) + G(1, range(nh, nch - 2))
            order += [("gm", 1, nch - 2), ("wait", "w2"), ("ac", 1, nch - 2)]
            order += [("dn", 0), ("dn", 1), ("wait", "xr")]
            ties = {(q // 5, nch - 6 + q % 5): q for q in range(10)}
        else:
            order = [("pk",), ("pq",), ("pjv",)]
            for n in range(NU + 1):
                order += [("qk", n)] if n < NU else G(0, range(3))
                if n >= 1:
                    order.append(("pv", n - 1))
                    if n - 1 == NG + 1:
                        order += [("wo", 0), ("ln2", 0)]
            order += G(0, [3]) + [("wo", 1), ("ln2", 1)] + G(0, range(4, nch)) + G(1, range(nch))
            order += [("dn", 0), ("dn", 1)]
            ties = {(1, 3 + q): q for q in range(10)}

        ot_rows = [[] for _ in range(NA)]
        h1 = [None] * NA
        hn = [None] * NA
        hid = [{} for _ in range(NA)]
        pend = {}
        mabs = xnf = done = None
        xn = None if first else xn_scr[i % 2]

        for t in order:
            op = t[0]
            if op == "start":
                for grp in groups.values():
                    for c_ in grp:
                        c_.start()
            elif op == "wait":
                for c_ in groups[t[1]]:
                    c_.wait()
            elif op == "ln0":
                xn = _ln(x_v[0:TB, :].astype(f32)).astype(bf16)
            elif op == "wvt":
                wvt_scr[...] = wqkv_v[:, 2 * D:3 * D].astype(f32).T.astype(bf16)
            elif op == "pa":
                qk_a = jnp.concatenate([_dot(xn[128 * u:128 * (u + 1)], wqkv_v[:, CA:2 * D]) for u in range(2)],
                                       axis=0)
            elif op == "pb":
                qk_b = _dot(xn, wqkv_v[:, CB:CA])
            elif op == "pc":
                qk_all = jnp.concatenate([_dot(xn, wqkv_v[:, 0:CB]), qk_b, qk_a], axis=1)
                put_k(qk_all[:, D:2 * D])
                put_q(qk_all[:, 0:D])
            elif op == "pk":
                put_k(_dot(xn, wqkv_v[:, D:2 * D]))
            elif op == "pq":
                put_q(_dot(xn, wqkv_v[:, 0:D]))
            elif op == "pjv":
                proj_v(xn)
            elif op == "qk":
                mabs = qk(t[1], mabs)
            elif op == "pv":
                ot_rows[t[1] // NG] += pv(t[1])
            elif op == "wo":
                h1[t[1]] = wo(t[1], ot_rows[t[1]])
            elif op == "ln2":
                hn[t[1]] = _ln(h1[t[1]]).astype(bf16)
            elif op in ("gu", "gm", "ac"):
                a, j = t[1], t[2]
                if op != "ac":
                    pend[a, j] = gu_mm(hn[a], j)
                if op != "gm":
                    tie = None
                    if (a, j) in ties:
                        if xnf is None:
                            nxt = pl.multiple_of(jnp.minimum(i + 1, NB - 1) * TB, TB)
                            xnf = _ln(x_v[pl.ds(nxt, TB), :].astype(f32))
                            xn_scr[(i + 1) % 2] = xnf.astype(bf16)
                        q = ties[a, j]
                        tie = xnf[128 * (q // 5):128 * (q // 5 + 1), 128 * (q % 5):128 * (q % 5 + 1)]
                    hid[a][j] = act(pend.pop((a, j)), tie)
            elif op == "dn":
                a = t[1]
                hcat = jnp.concatenate([hid[a][j] for j in range(nch)], axis=1)
                last = a == NA - 1
                dn = _dot_bal(hcat, w2_v[...], 4) if last else _dot(hcat, w2_v[...])
                outb = (h1[a] + dn).astype(bf16)
                if done is None:
                    ok = jnp.where(mabs <= SAFE, 1.0, 0.0)
                    done = jnp.logical_or(redo, jnp.min(ok) > 0.5)
                cuts = [0, D - 128, D] if last else [0, D]
                for c0, c1 in zip(cuts[:-1], cuts[1:]):
                    o_v[pl.ds(base + 128 * a, 128), c0:c1] = outb[:, c0:c1]
                    pl.when(done)(out_cp(base + 128 * a, c0, c1).start)
        return done

    def step(first, carry):
        i, r = carry
        done = body(first, i, r == 1)
        return jnp.where(done, i + 1, i), jnp.where(done, 0, 1)

    lax.while_loop(lambda c: c[0] < 1, functools.partial(step, True), (jnp.int32(0), jnp.int32(0)))
    lax.while_loop(lambda c: c[0] < NB, functools.partial(step, False), (jnp.int32(1), jnp.int32(0)))
    pltpu.make_async_copy(o_v, o_hbm, osem).wait()


@jax.jit
def pallas_sequential_preLN__sliding_block__glu_gated_swiglu__prompt_kernel(
    A_x: jax.Array,
    A_wqkv: jax.Array,
    A_wo: jax.Array,
    B_x: jax.Array,
    B_w1: jax.Array,
    B_w3: jax.Array,
    B_w2: jax.Array,
):
    del B_x
    hbm = pl.BlockSpec(memory_space=pl.ANY)
    out = pl.pallas_call(
        _kernel,
        in_specs=[hbm] * 6,
        out_specs=hbm,
        out_shape=jax.ShapeDtypeStruct((S, D), bf16),
        scratch_shapes=[
            pltpu.VMEM((S, D), bf16),
            pltpu.VMEM((S, D), bf16),
            pltpu.VMEM((D, 3 * D), bf16),
            pltpu.VMEM((D, D), bf16),
            pltpu.VMEM((F, D), bf16),
            pltpu.VMEM((F, D), bf16),
            pltpu.VMEM((F, D), bf16),
            pltpu.VMEM((D, D), bf16),
            pltpu.VMEM((2, TB, D), bf16),
            pltpu.VMEM((NG, S, 128), bf16),
            pltpu.VMEM((S // 128, H * 32, 128), bf16),
            pltpu.VMEM((NG, TB, 128), bf16),
            pltpu.VMEM((NU, 4, 288, 128), bf16),
            pltpu.VMEM((NU * 4, 1, 128), f32),
            pltpu.SemaphoreType.DMA((9,)),
            pltpu.SemaphoreType.DMA(()),
        ],
        compiler_params=pltpu.CompilerParams(vmem_limit_bytes=100 * 1024 * 1024),
    )(A_x.reshape(S, D), A_wqkv, A_wo, B_w1.T, B_w3.T, B_w2)
    return out.reshape(1, S, D)
```

```python
import functools
import math

import jax
import jax.numpy as jnp
from jax import lax
import jax.experimental.pallas as pl
import jax.experimental.pallas.tpu as pltpu

S, D, H, DH, W, F = 2048, 640, 32, 20, 256, 1728
NG = 8
GD = 80
TB = 256
NA = TB // 128
NB = S // TB
NU = NA * NG
NEG = -1e30
SAFE = 40.0
NT = (((1,), (1,)), ((), ()))
f32 = jnp.float32
bf16 = jnp.bfloat16
u32 = jnp.uint32
FM = 1664
FH = 896
CA, CB = 1024, 512
QSCALE = DH ** -0.5 * math.log2(math.e)


def _ln(x):
    m = jnp.mean(x, axis=-1, keepdims=True)
    xc = x - m
    v = jnp.mean(xc * xc, axis=-1, keepdims=True)
    return xc * lax.rsqrt(v + 1e-5)


def _group_tile(t, g):
    lo = GD * g
    j0, j1 = lo // 128, (lo + GD - 1) // 128
    a = t[:, 128 * j0:128 * (j0 + 1)]
    if j0 == j1:
        return a
    b = t[:, 128 * j1:128 * (j1 + 1)]
    lane = lax.broadcasted_iota(jnp.int32, a.shape, 1)
    return jnp.where(lane >= lo % 128, a, b)


def _silu_mul(g, u):
    return (g * u) * (0.5 * jnp.tanh(0.5 * g) + 0.5)


def _pack(x):
    return pltpu.bitcast(x.astype(bf16), u32)


def _bf(x):
    return pltpu.bitcast(x, bf16)


def _dot(a, b):
    return jnp.dot(a, b, preferred_element_type=f32)


def _dot_nt(a, b):
    return lax.dot_general(a, b, NT, preferred_element_type=f32)


def _dot_bal(lhs, w, nsplit):
    n = w.shape[1] - 128
    r = lhs.shape[0] // nsplit
    main = _dot(lhs, w[:, :n])
    last = [_dot(lhs[r * u:r * (u + 1)], w[:, n:]) for u in range(nsplit)]
    return jnp.concatenate([main, jnp.concatenate(last, axis=0)], axis=1)


def _kernel(x_hbm, wqkv_hbm, wo_hbm, w1t_hbm, w3t_hbm, w2_hbm, o_hbm,
            x_v, o_v, wqkv_v, wo_v, w1t_v, w3t_v, w2_v, wvt_scr, xn_scr, k_scr, vt_scr, q_scr, p_scr,
            m_scr, sems, osem):
    def cp(src, dst, s):
        return pltpu.make_async_copy(src, dst, sems.at[s])

    groups = {
        "x0": [cp(x_hbm.at[0:TB], x_v.at[0:TB], 0)],
        "a": [cp(wqkv_hbm.at[:, CA:2 * D], wqkv_v.at[:, CA:2 * D], 1)],
        "b": [cp(wqkv_hbm.at[:, CB:CA], wqkv_v.at[:, CB:CA], 2)],
        "c": [cp(wqkv_hbm.at[:, 0:CB], wqkv_v.at[:, 0:CB], 3)],
        "vo": [cp(wqkv_hbm.at[:, 2 * D:3 * D], wqkv_v.at[:, 2 * D:3 * D], 4), cp(wo_hbm, wo_v, 4)],
        "fa": [cp(w1t_hbm.at[0:FH], w1t_v.at[0:FH], 5), cp(w3t_hbm.at[0:FH], w3t_v.at[0:FH], 5)],
        "fb": [cp(w1t_hbm.at[FH:F], w1t_v.at[FH:F], 6), cp(w3t_hbm.at[FH:F], w3t_v.at[FH:F], 6),
               cp(x_hbm.at[TB:2 * TB], x_v.at[TB:2 * TB], 6)],
        "w2": [cp(w2_hbm, w2_v, 7)],
        "xr": [cp(x_hbm.at[2 * TB:S], x_v.at[2 * TB:S], 8)],
    }

    def out_cp(r, c0, c1):
        return pltpu.make_async_copy(o_v.at[pl.ds(r, 128), c0:c1], o_hbm.at[pl.ds(r, 128), c0:c1], osem)

    lane32 = lax.broadcasted_iota(jnp.int32, (32, 128), 1)
    row32 = lax.broadcasted_iota(jnp.int32, (32, 128), 0)
    old_valid = row32 > (lane32 % 32)
    lane16 = lax.broadcasted_iota(jnp.int32, (16, 128), 1)
    bit0 = (lane16 & 32) != 0
    bit1 = (lane16 & 64) != 0
    sub8 = lax.broadcasted_iota(jnp.int32, (8, 128), 0)
    zero16 = jnp.zeros((16, 128), u32)
    chunks = [(lo, lo + 128) for lo in range(0, FM, 128)] + [(FM, F)]
    nch = len(chunks)

    def body(first, i, redo):
        if first:
            base, hbase, tbase = 0, 0, 0
        else:
            base = pl.multiple_of(i * TB, TB)
            hbase = pl.multiple_of(i * (TB // 2), TB // 2)
            tbase = i * NA

        def put_k(k):
            for g in range(NG):
                k_scr[g, pl.ds(hbase, TB // 2), :] = _pack(_group_tile(k, g))

        def put_q(q):
            q = q * QSCALE
            for g in range(NG):
                q_scr[g] = _pack(_group_tile(q, g))

        def proj_v(xn, a0=0, a1=NA, g0=0, g1=NG):
            vt = _dot_nt(wvt_scr[GD * g0:GD * g1, :], xn[128 * a0:128 * a1])
            ones = jnp.ones((8, 128 * (a1 - a0)), f32)
            pieces = []
            for h in range(4 * (g1 - g0)):
                st = (DH * h) // 8 * 8
                pieces += [vt[st:st + 24], ones]
            vtp = _pack(jnp.concatenate(pieces, axis=0))
            for a in range(a0, a1):
                vt_scr[tbase + a, 64 * g0:64 * g1, :] = vtp[:, 128 * (a - a0):128 * (a - a0 + 1)]

        def qk(n, mabs):
            a, g = n // NG, n % NG
            rel = (lane16 + (128 - (GD * g) % 128)) % 128
            for c in range(4):
                q0 = 128 * a + 32 * c
                un = n * 4 + c
                qu = q_scr[g, q0 // 2:q0 // 2 + 16, :]
                wb = []
                for b in range(4):
                    h = b ^ c
                    wb.append(jnp.where((rel >= DH * h) & (rel < DH * (h + 1)), qu, zero16))
                wq = _bf(jnp.concatenate(wb, axis=0))
                mref = jnp.where(redo, m_scr[un], 0.0)
                if first:
                    st = _dot_nt(_bf(k_scr[g, 0:q0 // 2 + 16, :]), wq)
                    diag = jnp.where(old_valid, NEG, st[q0:q0 + 32])
                    sc = diag if q0 == 0 else jnp.concatenate([st[0:q0], diag], axis=0)
                    p_scr[n, c, 0:q0 // 2 + 16, :] = _pack(jnp.exp2(sc - mref))
                else:
                    r0 = pl.multiple_of(hbase + (q0 - W) // 2, 16)
                    st = _dot_nt(_bf(k_scr[g, pl.ds(r0, 144), :]), wq)
                    edge = jnp.where(old_valid, st[0:32], st[256:288])
                    sc = jnp.concatenate([st[32:256], edge], axis=0)
                    pe = jnp.exp2(edge - mref)
                    p_scr[n, c, 0:16, :] = _pack(jnp.where(old_valid, pe, 0.0))
                    p_scr[n, c, 128:144, :] = _pack(jnp.where(old_valid, 0.0, pe))
                    p_scr[n, c, 16:128, :] = _pack(jnp.exp2(st[32:256] - mref))
                m = jnp.max(sc, axis=0, keepdims=True)
                m_scr[un] = m
                am = jnp.abs(m)
                mabs = am if mabs is None else jnp.maximum(mabs, am)
            return mabs

        def sel(mask, t, f):
            if t is None and f is None:
                return None
            return jnp.where(mask, zero16 if t is None else t, zero16 if f is None else f)

        def pv(n):
            a, g = n // NG, n % NG
            if first:
                nblk = 4 * (a + 1)
                blk = lambda c, j: (p_scr[n, c, 16 * j:16 * j + 16, :] if j <= 4 * a + c else None)
                tiles = list(range(a + 1))
            else:
                nblk = 12
                blk = lambda c, j: (p_scr[n, c, 16 * (j - c):16 * (j - c) + 16, :] if c <= j <= c + 8 else None)
                tiles = [tbase + a - 2 + t for t in range(3)]
            outs = [[], [], [], []]
            for j in range(nblk):
                pts = [blk(c, j) for c in range(4)]
                y = [sel(bit0, pts[c ^ 1], pts[c]) for c in range(4)]
                for h in range(4):
                    z = sel(bit1, y[h ^ 2], y[h])
                    outs[h].append(zero16 if z is None else z)
            ots = [None] * 4
            for ti, t in enumerate(tiles):
                for h in range(4):
                    hh = 4 * g + h
                    pth = _bf(jnp.concatenate(outs[h][4 * ti:4 * ti + 4], axis=0))
                    d = _dot(_bf(vt_scr[t, 16 * hh:16 * hh + 16, :]), pth)
                    ots[h] = d if ots[h] is None else ots[h] + d
            on = []
            for h in range(4):
                r = 1.0 / ots[h][24:32]
                on.append([ots[h][0:8] * r, ots[h][8:16] * r, ots[h][16:24] * r])
            return [on[0][0], on[0][1], jnp.where(sub8 < 4, on[0][2], on[1][0]), on[1][1], on[1][2],
                    on[2][0], on[2][1], jnp.where(sub8 < 4, on[2][2], on[3][0]), on[3][1], on[3][2]]

        def wo(a, ot_rows):
            mt = jnp.concatenate(ot_rows, axis=0).T
            col = lax.broadcasted_iota(jnp.int32, (32, D), 1)
            hb0 = (col // DH) % 2 == 1
            hb1 = (col // (2 * DH)) % 2 == 1
            rb = [mt[32 * b:32 * (b + 1)] for b in range(4)]
            y = [jnp.where(hb0, rb[c ^ 1], rb[c]) for c in range(4)]
            z = [jnp.where(hb1, y[c ^ 2], y[c]) for c in range(4)]
            o = jnp.concatenate(z, axis=0).astype(bf16)
            return x_v[pl.ds(base + 128 * a, 128), :].astype(f32) + _dot(o, wo_v[...])

        def gu_mm(hn, j):
            lo, hi = chunks[j]
            if lo == FM:
                return (_dot_nt(hn, jnp.concatenate([w1t_v[FM:F, :], w3t_v[FM:F, :]], axis=0)),)
            return _dot_nt(hn, w1t_v[lo:hi, :]), _dot_nt(hn, w3t_v[lo:hi, :])

        def act(gu_, tie):
            if len(gu_) == 1:
                t = gu_[0]
                return _silu_mul(t, pltpu.roll(t, 64, 1))[:, 0:64].astype(bf16)
            r = _silu_mul(*gu_)
            if tie is not None:
                r = jnp.where(i > NB, tie, r)
            return r.astype(bf16)

        G = lambda a, js: [("gu", a, j) for j in js]
        if first:
            nh = FH // 128
            order = [("start",), ("wait", "x0"), ("ln0",), ("wait", "a"), ("pa",), ("wait", "b"), ("pb",),
                     ("wait", "c"), ("pc",)]
            order += [("qk", n) for n in list(range(NG, NU - 2)) + list(range(NG))]
            order += [("wait", "vo"), ("wvt",), ("qk", NU - 2), ("qk", NU - 1)]
            P = lambda *ns: [("pv", n) for n in ns]
            V = lambda a, g0, g1: [("pjv", a, a + 1, g0, g1)]
            order += V(0, 0, 4) + V(1, 0, 4) + P(0, 1) + V(0, 4, 8) + P(2, 3, 8, 9) + V(1, 4, 6)
            order += P(4, 5, 6, 7, 10) + V(1, 6, 8) + P(11, 12, 13, 14, 15)
            order += [("wo", 0), ("ln2", 0), ("wo", 1), ("wait", "fa"), ("ln2", 1)]
            order += G(0, range(nh)) + G(1, range(nh - 1)) + [("gm", 1, nh - 1), ("wait", "fb"), ("ac", 1, nh - 1)]
            order += G(0, [nch - 1]) + G(1, [nch - 1])
            order += G(0, range(nh, nch - 1)) + G(1, range(nh, nch - 2))
            order += [("gm", 1, nch - 2), ("wait", "w2"), ("ac", 1, nch - 2)]
            order += [("dn", 0), ("dn", 1), ("wait", "xr")]
            ties = {(q // 5, nch - 6 + q % 5): q for q in range(10)}
        else:
            order = [("pk",), ("pq",), ("pjv",)]
            for n in range(NU + 1):
                order += [("qk", n)] if n < NU else G(0, range(3))
                if n >= 1:
                    order.append(("pv", n - 1))
                    if n - 1 == NG + 1:
                        order += [("wo", 0), ("ln2", 0)]
            order += G(0, [3]) + [("wo", 1), ("ln2", 1)] + G(0, range(4, nch)) + G(1, range(nch))
            order += [("dn", 0), ("dn", 1)]
            ties = {(1, 3 + q): q for q in range(10)}

        ot_rows = [[] for _ in range(NA)]
        h1 = [None] * NA
        hn = [None] * NA
        hid = [{} for _ in range(NA)]
        pend = {}
        mabs = xnf = done = None
        xn = None if first else xn_scr[i % 2]

        for t in order:
            op = t[0]
            if op == "start":
                for grp in groups.values():
                    for c_ in grp:
                        c_.start()
            elif op == "wait":
                for c_ in groups[t[1]]:
                    c_.wait()
            elif op == "ln0":
                xn = _ln(x_v[0:TB, :].astype(f32)).astype(bf16)
            elif op == "wvt":
                wvt_scr[...] = wqkv_v[:, 2 * D:3 * D].astype(f32).T.astype(bf16)
            elif op == "pa":
                qk_a = jnp.concatenate([_dot(xn[128 * u:128 * (u + 1)], wqkv_v[:, CA:2 * D]) for u in range(2)],
                                       axis=0)
            elif op == "pb":
                qk_b = _dot(xn, wqkv_v[:, CB:CA])
            elif op == "pc":
                qk_all = jnp.concatenate([_dot(xn, wqkv_v[:, 0:CB]), qk_b, qk_a], axis=1)
                put_k(qk_all[:, D:2 * D])
                put_q(qk_all[:, 0:D])
            elif op == "pk":
                put_k(_dot(xn, wqkv_v[:, D:2 * D]))
            elif op == "pq":
                put_q(_dot(xn, wqkv_v[:, 0:D]))
            elif op == "pjv":
                proj_v(xn, *t[1:])
            elif op == "qk":
                mabs = qk(t[1], mabs)
            elif op == "pv":
                ot_rows[t[1] // NG] += pv(t[1])
            elif op == "wo":
                h1[t[1]] = wo(t[1], ot_rows[t[1]])
            elif op == "ln2":
                hn[t[1]] = _ln(h1[t[1]]).astype(bf16)
            elif op in ("gu", "gm", "ac"):
                a, j = t[1], t[2]
                if op != "ac":
                    pend[a, j] = gu_mm(hn[a], j)
                if op != "gm":
                    tie = None
                    if (a, j) in ties:
                        if xnf is None:
                            nxt = pl.multiple_of(jnp.minimum(i + 1, NB - 1) * TB, TB)
                            xnf = _ln(x_v[pl.ds(nxt, TB), :].astype(f32))
                            xn_scr[(i + 1) % 2] = xnf.astype(bf16)
                        q = ties[a, j]
                        tie = xnf[128 * (q // 5):128 * (q // 5 + 1), 128 * (q % 5):128 * (q % 5 + 1)]
                    hid[a][j] = act(pend.pop((a, j)), tie)
            elif op == "dn":
                a = t[1]
                hcat = jnp.concatenate([hid[a][j] for j in range(nch)], axis=1)
                last = a == NA - 1
                dn = _dot_bal(hcat, w2_v[...], 4) if last else _dot(hcat, w2_v[...])
                outb = (h1[a] + dn).astype(bf16)
                if done is None:
                    ok = jnp.where(mabs <= SAFE, 1.0, 0.0)
                    done = jnp.logical_or(redo, jnp.min(ok) > 0.5)
                cuts = [0, D - 128, D] if last else [0, D]
                for c0, c1 in zip(cuts[:-1], cuts[1:]):
                    o_v[pl.ds(base + 128 * a, 128), c0:c1] = outb[:, c0:c1]
                    pl.when(done)(out_cp(base + 128 * a, c0, c1).start)
        return done

    def step(first, carry):
        i, r = carry
        done = body(first, i, r == 1)
        return jnp.where(done, i + 1, i), jnp.where(done, 0, 1)

    lax.while_loop(lambda c: c[0] < 1, functools.partial(step, True), (jnp.int32(0), jnp.int32(0)))
    lax.while_loop(lambda c: c[0] < NB, functools.partial(step, False), (jnp.int32(1), jnp.int32(0)))
    pltpu.make_async_copy(o_v, o_hbm, osem).wait()


@jax.jit
def pallas_sequential_preLN__sliding_block__glu_gated_swiglu__prompt_kernel(
    A_x: jax.Array,
    A_wqkv: jax.Array,
    A_wo: jax.Array,
    B_x: jax.Array,
    B_w1: jax.Array,
    B_w3: jax.Array,
    B_w2: jax.Array,
):
    del B_x
    hbm = pl.BlockSpec(memory_space=pl.ANY)
    out = pl.pallas_call(
        _kernel,
        in_specs=[hbm] * 6,
        out_specs=hbm,
        out_shape=jax.ShapeDtypeStruct((S, D), bf16),
        scratch_shapes=[
            pltpu.VMEM((S, D), bf16),
            pltpu.VMEM((S, D), bf16),
            pltpu.VMEM((D, 3 * D), bf16),
            pltpu.VMEM((D, D), bf16),
            pltpu.VMEM((F, D), bf16),
            pltpu.VMEM((F, D), bf16),
            pltpu.VMEM((F, D), bf16),
            pltpu.VMEM((D, D), bf16),
            pltpu.VMEM((2, TB, D), bf16),
            pltpu.VMEM((NG, S // 2, 128), u32),
            pltpu.VMEM((S // 128, H * 16, 128), u32),
            pltpu.VMEM((NG, TB // 2, 128), u32),
            pltpu.VMEM((NU, 4, 144, 128), u32),
            pltpu.VMEM((NU * 4, 1, 128), f32),
            pltpu.SemaphoreType.DMA((9,)),
            pltpu.SemaphoreType.DMA(()),
        ],
        compiler_params=pltpu.CompilerParams(vmem_limit_bytes=100 * 1024 * 1024),
    )(A_x.reshape(S, D), A_wqkv, A_wo, B_w1.T, B_w3.T, B_w2)
    return out.reshape(1, S, D)
```

```python
import functools
import math

import jax
import jax.numpy as jnp
from jax import lax
import jax.experimental.pallas as pl
import jax.experimental.pallas.tpu as pltpu

S, D, H, DH, W, F = 2048, 640, 32, 20, 256, 1728
NG = 8
GD = 80
TB = 256
NA = TB // 128
NB = S // TB
NU = NA * NG
NEG = -1e30
SAFE = 40.0
NT = (((1,), (1,)), ((), ()))
f32 = jnp.float32
bf16 = jnp.bfloat16
u32 = jnp.uint32
FM = 1664
FH = 896
CA, CB = 1024, 512
QSCALE = DH ** -0.5 * math.log2(math.e)


def _ln(x):
    m = jnp.mean(x, axis=-1, keepdims=True)
    xc = x - m
    v = jnp.mean(xc * xc, axis=-1, keepdims=True)
    return xc * lax.rsqrt(v + 1e-5)


def _group_tile(t, g):
    lo = GD * g
    j0, j1 = lo // 128, (lo + GD - 1) // 128
    a = t[:, 128 * j0:128 * (j0 + 1)]
    if j0 == j1:
        return a
    b = t[:, 128 * j1:128 * (j1 + 1)]
    lane = lax.broadcasted_iota(jnp.int32, a.shape, 1)
    return jnp.where(lane >= lo % 128, a, b)


def _silu_mul(g, u):
    return (g * (0.5 * jnp.tanh(0.5 * g) + 0.5)) * u


def _pack(x):
    return pltpu.bitcast(x.astype(bf16), u32)


def _bf(x):
    return pltpu.bitcast(x, bf16)


def _dot(a, b):
    return jnp.dot(a, b, preferred_element_type=f32)


def _dot_nt(a, b):
    return lax.dot_general(a, b, NT, preferred_element_type=f32)


def _dot_bal(lhs, w, nsplit):
    n = w.shape[1] - 128
    r = lhs.shape[0] // nsplit
    main = _dot(lhs, w[:, :n])
    last = [_dot(lhs[r * u:r * (u + 1)], w[:, n:]) for u in range(nsplit)]
    return jnp.concatenate([main, jnp.concatenate(last, axis=0)], axis=1)


def _kernel(x_hbm, wqkv_hbm, wo_hbm, w1t_hbm, w3t_hbm, w2_hbm, o_hbm,
            x_v, o_v, wqkv_v, wo_v, w1t_v, w3t_v, w2_v, wvt_scr, xn_scr, k_scr, vt_scr, q_scr, p_scr,
            m_scr, sems, osem):
    def cp(src, dst, s):
        return pltpu.make_async_copy(src, dst, sems.at[s])

    groups = {
        "x0": [cp(x_hbm.at[0:TB], x_v.at[0:TB], 0)],
        "a": [cp(wqkv_hbm.at[:, CA:2 * D], wqkv_v.at[:, CA:2 * D], 1)],
        "b": [cp(wqkv_hbm.at[:, CB:CA], wqkv_v.at[:, CB:CA], 2)],
        "c": [cp(wqkv_hbm.at[:, 0:CB], wqkv_v.at[:, 0:CB], 3)],
        "vo": [cp(wqkv_hbm.at[:, 2 * D:3 * D], wqkv_v.at[:, 2 * D:3 * D], 4), cp(wo_hbm, wo_v, 4)],
        "fa": [cp(w1t_hbm.at[0:FH], w1t_v.at[0:FH], 5), cp(w3t_hbm.at[0:FH], w3t_v.at[0:FH], 5)],
        "fb": [cp(w1t_hbm.at[FH:F], w1t_v.at[FH:F], 6), cp(w3t_hbm.at[FH:F], w3t_v.at[FH:F], 6),
               cp(x_hbm.at[TB:2 * TB], x_v.at[TB:2 * TB], 6)],
        "w2": [cp(w2_hbm, w2_v, 7)],
        "xr": [cp(x_hbm.at[2 * TB:S], x_v.at[2 * TB:S], 8)],
    }

    def out_cp(r, c0, c1):
        return pltpu.make_async_copy(o_v.at[pl.ds(r, 128), c0:c1], o_hbm.at[pl.ds(r, 128), c0:c1], osem)

    lane32 = lax.broadcasted_iota(jnp.int32, (32, 128), 1)
    row32 = lax.broadcasted_iota(jnp.int32, (32, 128), 0)
    old_valid = row32 > (lane32 % 32)
    lane16 = lax.broadcasted_iota(jnp.int32, (16, 128), 1)
    bit0 = (lane16 & 32) != 0
    bit1 = (lane16 & 64) != 0
    sub8 = lax.broadcasted_iota(jnp.int32, (8, 128), 0)
    zero16 = jnp.zeros((16, 128), u32)
    chunks = [(lo, lo + 128) for lo in range(0, FM, 128)] + [(FM, F)]
    nch = len(chunks)

    def body(first, i, redo):
        if first:
            base, hbase, tbase = 0, 0, 0
        else:
            base = pl.multiple_of(i * TB, TB)
            hbase = pl.multiple_of(i * (TB // 2), TB // 2)
            tbase = i * NA

        def put_k(k):
            for g in range(NG):
                k_scr[g, pl.ds(hbase, TB // 2), :] = _pack(_group_tile(k, g))

        def put_q(q):
            q = q * QSCALE
            for g in range(NG):
                q_scr[g] = _pack(_group_tile(q, g))

        def proj_v(xn, a0=0, a1=NA, g0=0, g1=NG):
            vt = _dot_nt(wvt_scr[GD * g0:GD * g1, :], xn[128 * a0:128 * a1])
            ones = jnp.ones((8, 128 * (a1 - a0)), f32)
            pieces = []
            for h in range(4 * (g1 - g0)):
                st = (DH * h) // 8 * 8
                pieces += [vt[st:st + 24], ones]
            vtp = _pack(jnp.concatenate(pieces, axis=0))
            for a in range(a0, a1):
                vt_scr[tbase + a, 64 * g0:64 * g1, :] = vtp[:, 128 * (a - a0):128 * (a - a0 + 1)]

        def qk(n, mabs):
            a, g = n // NG, n % NG
            rel = (lane16 + (128 - (GD * g) % 128)) % 128
            for c in range(4):
                q0 = 128 * a + 32 * c
                un = n * 4 + c
                qu = q_scr[g, q0 // 2:q0 // 2 + 16, :]
                wb = []
                for b in range(4):
                    h = b ^ c
                    wb.append(jnp.where((rel >= DH * h) & (rel < DH * (h + 1)), qu, zero16))
                wq = _bf(jnp.concatenate(wb, axis=0))
                mref = jnp.where(redo, m_scr[un:un + 1, :], 0.0)
                if first:
                    st = _dot_nt(_bf(k_scr[g, 0:q0 // 2 + 16, :]), wq)
                    diag = jnp.where(old_valid, NEG, st[q0:q0 + 32])
                    sc = diag if q0 == 0 else jnp.concatenate([st[0:q0], diag], axis=0)
                    p_scr[n, c, 0:q0 // 2 + 16, :] = _pack(jnp.exp2(sc - mref))
                else:
                    r0 = pl.multiple_of(hbase + (q0 - W) // 2, 16)
                    st = _dot_nt(_bf(k_scr[g, pl.ds(r0, 144), :]), wq)
                    edge = jnp.where(old_valid, st[0:32], st[256:288])
                    sc = jnp.concatenate([st[32:256], edge], axis=0)
                    pe = jnp.exp2(edge - mref)
                    p_scr[n, c, 0:16, :] = _pack(jnp.where(old_valid, pe, 0.0))
                    p_scr[n, c, 128:144, :] = _pack(jnp.where(old_valid, 0.0, pe))
                    p_scr[n, c, 16:128, :] = _pack(jnp.exp2(st[32:256] - mref))
                m = jnp.max(sc, axis=0, keepdims=True)
                m_scr[un:un + 1, :] = m
                am = jnp.abs(m)
                mabs = am if mabs is None else jnp.maximum(mabs, am)
            return mabs

        def sel(mask, t, f):
            if t is None and f is None:
                return None
            return jnp.where(mask, zero16 if t is None else t, zero16 if f is None else f)

        def pv(n):
            a, g = n // NG, n % NG
            if first:
                nblk = 4 * (a + 1)
                blk = lambda c, j: (p_scr[n, c, 16 * j:16 * j + 16, :] if j <= 4 * a + c else None)
                tiles = list(range(a + 1))
            else:
                nblk = 12
                blk = lambda c, j: (p_scr[n, c, 16 * (j - c):16 * (j - c) + 16, :] if c <= j <= c + 8 else None)
                tiles = [tbase + a - 2 + t for t in range(3)]
            outs = [[], [], [], []]
            for j in range(nblk):
                pts = [blk(c, j) for c in range(4)]
                y = [sel(bit0, pts[c ^ 1], pts[c]) for c in range(4)]
                for h in range(4):
                    z = sel(bit1, y[h ^ 2], y[h])
                    outs[h].append(zero16 if z is None else z)
            ots = [None] * 4
            for ti, t in enumerate(tiles):
                for h in range(4):
                    hh = 4 * g + h
                    pth = _bf(jnp.concatenate(outs[h][4 * ti:4 * ti + 4], axis=0))
                    d = _dot(_bf(vt_scr[t, 16 * hh:16 * hh + 16, :]), pth)
                    ots[h] = d if ots[h] is None else ots[h] + d
            on = []
            for h in range(4):
                r = 1.0 / ots[h][24:32]
                on.append([ots[h][0:8] * r, ots[h][8:16] * r, ots[h][16:24] * r])
            return [on[0][0], on[0][1], jnp.where(sub8 < 4, on[0][2], on[1][0]), on[1][1], on[1][2],
                    on[2][0], on[2][1], jnp.where(sub8 < 4, on[2][2], on[3][0]), on[3][1], on[3][2]]

        def wo(a, ot_rows):
            mt = jnp.concatenate(ot_rows, axis=0).T
            col = lax.broadcasted_iota(jnp.int32, (32, D), 1)
            hb0 = (col // DH) % 2 == 1
            hb1 = (col // (2 * DH)) % 2 == 1
            rb = [mt[32 * b:32 * (b + 1)] for b in range(4)]
            y = [jnp.where(hb0, rb[c ^ 1], rb[c]) for c in range(4)]
            z = [jnp.where(hb1, y[c ^ 2], y[c]) for c in range(4)]
            o = jnp.concatenate(z, axis=0).astype(bf16)
            return x_v[pl.ds(base + 128 * a, 128), :].astype(f32) + _dot(o, wo_v[...])

        def gu_mm(hn, j):
            lo, hi = chunks[j]
            if lo == FM:
                return (_dot_nt(hn, jnp.concatenate([w1t_v[FM:F, :], w3t_v[FM:F, :]], axis=0)),)
            return _dot_nt(hn, w1t_v[lo:hi, :]), _dot_nt(hn, w3t_v[lo:hi, :])

        def act(gu_, tie):
            if len(gu_) == 1:
                t = gu_[0]
                return _silu_mul(t, pltpu.roll(t, 64, 1))[:, 0:64].astype(bf16)
            r = _silu_mul(*gu_)
            if tie is not None:
                r = jnp.where(i > NB, tie, r)
            return r.astype(bf16)

        G = lambda a, js: [("gu", a, j) for j in js]
        if first:
            nh = FH // 128
            order = [("start",), ("wait", "x0"), ("ln0",), ("wait", "a"), ("pa",), ("wait", "b"), ("pb",),
                     ("wait", "c"), ("pc",)]
            order += [("qk", n) for n in list(range(NG, NU - 2)) + list(range(NG))]
            order += [("wait", "vo"), ("wvt",), ("qk", NU - 2), ("qk", NU - 1)]
            P = lambda *ns: [("pv", n) for n in ns]
            V = lambda a, g0, g1: [("pjv", a, a + 1, g0, g1)]
            order += V(0, 0, 4) + V(1, 0, 4) + P(0, 1) + V(0, 4, 8) + P(2, 3, 8, 9) + V(1, 4, 6)
            order += P(4, 5, 6, 7, 10) + V(1, 6, 8) + P(11, 12, 13, 14, 15)
            order += [("wo", 0), ("ln2", 0), ("wo", 1), ("wait", "fa"), ("ln2", 1)]
            order += G(0, range(nh)) + G(1, range(nh - 1)) + [("gm", 1, nh - 1), ("wait", "fb"), ("ac", 1, nh - 1)]
            order += G(0, [nch - 1]) + G(1, [nch - 1])
            order += G(0, range(nh, nch - 1)) + G(1, range(nh, nch - 2))
            order += [("gm", 1, nch - 2), ("wait", "w2"), ("ac", 1, nch - 2)]
            order += [("dn", 0), ("dn", 1), ("wait", "xr")]
            ties = {(q // 5, nch - 6 + q % 5): q for q in range(10)}
        else:
            order = [("pk",), ("pq",), ("pjv",)]
            for n in range(NU + 1):
                order += [("qk", n)] if n < NU else G(0, range(3))
                if n >= 1:
                    order.append(("pv", n - 1))
                    if n - 1 == NG + 1:
                        order += [("wo", 0), ("ln2", 0)]
            order += G(0, [3]) + [("wo", 1), ("ln2", 1)] + G(0, range(4, nch)) + G(1, range(nch))
            order += [("dn", 0), ("dn", 1)]
            ties = {(1, 3 + q): q for q in range(10)}

        ot_rows = [[] for _ in range(NA)]
        h1 = [None] * NA
        hn = [None] * NA
        hid = [{} for _ in range(NA)]
        pend = {}
        mabs = xnf = done = None
        xn = None if first else xn_scr[i % 2]

        for t in order:
            op = t[0]
            if op == "start":
                for grp in groups.values():
                    for c_ in grp:
                        c_.start()
            elif op == "wait":
                for c_ in groups[t[1]]:
                    c_.wait()
            elif op == "ln0":
                xn = _ln(x_v[0:TB, :].astype(f32)).astype(bf16)
            elif op == "wvt":
                wvt_scr[...] = wqkv_v[:, 2 * D:3 * D].astype(f32).T.astype(bf16)
            elif op == "pa":
                qk_a = jnp.concatenate([_dot(xn[128 * u:128 * (u + 1)], wqkv_v[:, CA:2 * D]) for u in range(2)],
                                       axis=0)
            elif op == "pb":
                qk_b = _dot(xn, wqkv_v[:, CB:CA])
            elif op == "pc":
                qk_all = jnp.concatenate([_dot(xn, wqkv_v[:, 0:CB]), qk_b, qk_a], axis=1)
                put_k(qk_all[:, D:2 * D])
                put_q(qk_all[:, 0:D])
            elif op == "pk":
                put_k(_dot(xn, wqkv_v[:, D:2 * D]))
            elif op == "pq":
                put_q(_dot(xn, wqkv_v[:, 0:D]))
            elif op == "pjv":
                proj_v(xn, *t[1:])
            elif op == "qk":
                mabs = qk(t[1], mabs)
            elif op == "pv":
                ot_rows[t[1] // NG] += pv(t[1])
            elif op == "wo":
                h1[t[1]] = wo(t[1], ot_rows[t[1]])
            elif op == "ln2":
                hn[t[1]] = _ln(h1[t[1]]).astype(bf16)
            elif op in ("gu", "gm", "ac"):
                a, j = t[1], t[2]
                if op != "ac":
                    pend[a, j] = gu_mm(hn[a], j)
                if op != "gm":
                    tie = None
                    if (a, j) in ties:
                        if xnf is None:
                            nxt = pl.multiple_of(jnp.minimum(i + 1, NB - 1) * TB, TB)
                            xnf = _ln(x_v[pl.ds(nxt, TB), :].astype(f32))
                            xn_scr[(i + 1) % 2] = xnf.astype(bf16)
                        q = ties[a, j]
                        tie = xnf[128 * (q // 5):128 * (q // 5 + 1), 128 * (q % 5):128 * (q % 5 + 1)]
                    hid[a][j] = act(pend.pop((a, j)), tie)
            elif op == "dn":
                a = t[1]
                hcat = jnp.concatenate([hid[a][j] for j in range(nch)], axis=1)
                last = a == NA - 1
                dn = _dot_bal(hcat, w2_v[...], 4) if last else _dot(hcat, w2_v[...])
                outb = (h1[a] + dn).astype(bf16)
                if done is None:
                    ok = jnp.where(mabs <= SAFE, 1.0, 0.0)
                    done = jnp.logical_or(redo, jnp.min(ok) > 0.5)
                cuts = [0, D - 128, D] if last else [0, D]
                for c0, c1 in zip(cuts[:-1], cuts[1:]):
                    o_v[pl.ds(base + 128 * a, 128), c0:c1] = outb[:, c0:c1]
                    pl.when(done)(out_cp(base + 128 * a, c0, c1).start)
        return done

    def step(first, carry):
        i, r = carry
        done = body(first, i, r == 1)
        return jnp.where(done, i + 1, i), jnp.where(done, 0, 1)

    m_scr[...] = jnp.zeros(m_scr.shape, f32)
    lax.while_loop(lambda c: c[0] < 1, functools.partial(step, True), (jnp.int32(0), jnp.int32(0)))
    lax.while_loop(lambda c: c[0] < NB, functools.partial(step, False), (jnp.int32(1), jnp.int32(0)))
    pltpu.make_async_copy(o_v, o_hbm, osem).wait()


@jax.jit
def pallas_sequential_preLN__sliding_block__glu_gated_swiglu__prompt_kernel(
    A_x: jax.Array,
    A_wqkv: jax.Array,
    A_wo: jax.Array,
    B_x: jax.Array,
    B_w1: jax.Array,
    B_w3: jax.Array,
    B_w2: jax.Array,
):
    del B_x
    hbm = pl.BlockSpec(memory_space=pl.ANY)
    out = pl.pallas_call(
        _kernel,
        in_specs=[hbm] * 6,
        out_specs=hbm,
        out_shape=jax.ShapeDtypeStruct((S, D), bf16),
        scratch_shapes=[
            pltpu.VMEM((S, D), bf16),
            pltpu.VMEM((S, D), bf16),
            pltpu.VMEM((D, 3 * D), bf16),
            pltpu.VMEM((D, D), bf16),
            pltpu.VMEM((F, D), bf16),
            pltpu.VMEM((F, D), bf16),
            pltpu.VMEM((F, D), bf16),
            pltpu.VMEM((D, D), bf16),
            pltpu.VMEM((2, TB, D), bf16),
            pltpu.VMEM((NG, S // 2, 128), u32),
            pltpu.VMEM((S // 128, H * 16, 128), u32),
            pltpu.VMEM((NG, TB // 2, 128), u32),
            pltpu.VMEM((NU, 4, 144, 128), u32),
            pltpu.VMEM((NU * 4, 128), f32),
            pltpu.SemaphoreType.DMA((9,)),
            pltpu.SemaphoreType.DMA(()),
        ],
        compiler_params=pltpu.CompilerParams(vmem_limit_bytes=100 * 1024 * 1024),
    )(A_x.reshape(S, D), A_wqkv, A_wo, B_w1.T, B_w3.T, B_w2)
    return out.reshape(1, S, D)
```
